```python
import os as _os
_os.environ.setdefault("JAX_PLATFORMS", "cpu")
import jax
import jax.numpy as jnp

def _softmax(x, axis=-1):
    return jax.nn.softmax(x, axis=axis)
def _gelu(x):
    return jax.nn.gelu(x, approximate=True)
def _silu(x):
    return jax.nn.silu(x)
def _sigmoid(x):
    return jax.nn.sigmoid(x)
def _layernorm(x, axis=-1, eps=1e-5):
    m = jnp.mean(x, axis=axis, keepdims=True)
    v = jnp.var(x, axis=axis, keepdims=True)
    return (x - m) / jnp.sqrt(v + eps)
def _scatter_add(tgt, idx, src, axis=0):
    return tgt.at[idx].add(src)
def _segment_sum(src, seg, n):
    return jax.ops.segment_sum(src, seg, n)
class _Rng:
    def __init__(self, key):
        self._k = key
    def _next(self):
        self._k, sub = jax.random.split(self._k)
        return sub
    def normal(self, shape):
        return jax.random.normal(self._next(), shape, dtype=jnp.bfloat16)
    def randint(self, lo, hi, shape):
        return jax.random.randint(self._next(), shape, lo, hi, dtype=jnp.int32)
    def uniform(self, shape, lo=0.0, hi=1.0):
        return jax.random.uniform(self._next(), shape, jnp.bfloat16, lo, hi)
    def permutation(self, n):
        return jax.random.permutation(self._next(), n)


kernel_name = 'concat_heads__sliding_block_cached__sliding_block_cached__decode'

def setup_inputs():
    _rng = _Rng(jax.random.key(int.from_bytes(__import__("os").urandom(4), "little")))
    _w = (lambda a: (lambda t: t.astype(jnp.bfloat16) if jnp.issubdtype(t.dtype, jnp.floating) else t)(jnp.asarray(a)))
    def _A_setup():
        B, Sq, D = 4, 1, 576
        Hq, Hkv, Sk, Dh = 32, 16, 8192, 128
        assert Hq % Hkv == 0, (Hq, Hkv)
        return {
            "x": _w((lambda *s: _rng.normal(s) * 0.8)(B, Sq, D)),
            "k_cache": _w((lambda *s: _rng.normal(s) * 0.8)(B, Hkv, Sk, Dh)),
            "v_cache": _w((lambda *s: _rng.normal(s) * 0.05)(B, Hkv, Sk, Dh)),
            "wq": _w((lambda *s: _rng.normal(s) * 0.8)(D, Hq * Dh) * (D ** -0.5)),
            "wo": _w((lambda *s: _rng.normal(s) * 0.05)(Hq * Dh, D) * ((Hq * Dh) ** -0.5)),
        }
    _A_in = _A_setup()

    def _B_setup():
        B, Sq, D = 4, 1, 576
        Hq, Hkv, Sk, Dh = 32, 16, 8192, 128
        assert Hq % Hkv == 0, (Hq, Hkv)
        return {
            "x": _w((lambda *s: _rng.normal(s) * 0.8)(B, Sq, D)),
            "k_cache": _w((lambda *s: _rng.normal(s) * 0.8)(B, Hkv, Sk, Dh)),
            "v_cache": _w((lambda *s: _rng.normal(s) * 0.05)(B, Hkv, Sk, Dh)),
            "wq": _w((lambda *s: _rng.normal(s) * 0.8)(D, Hq * Dh) * (D ** -0.5)),
            "wo": _w((lambda *s: _rng.normal(s) * 0.05)(Hq * Dh, D) * ((Hq * Dh) ** -0.5)),
        }
    _B_in = _B_setup()

    return {
        "A_x": _A_in["x"],
        "A_k_cache": _A_in["k_cache"],
        "A_v_cache": _A_in["v_cache"],
        "A_wq": _A_in["wq"],
        "A_wo": _A_in["wo"],
        "B_x": _B_in["x"],
        "B_k_cache": _B_in["k_cache"],
        "B_v_cache": _B_in["v_cache"],
        "B_wq": _B_in["wq"],
        "B_wo": _B_in["wo"],
    }

def reference(A_x, A_k_cache, A_v_cache, A_wq, A_wo, B_x, B_k_cache, B_v_cache, B_wq, B_wo):
    def _A_ref(x, k_cache, v_cache, wq, wo):
        B, Sq, D = x.shape
        Hq, Dh = 32, 128
        Hkv, Sk = k_cache.shape[1], k_cache.shape[2]
        W = min(4096, max(256, Sk // 4))
        rep = Hq // Hkv
        q = (lambda x, *d: x.transpose(*d))((x @ wq).reshape(B, Sq, Hq, Dh), 0, 2, 1, 3)
        k = jnp.repeat(k_cache[:, :, Sk - W:, :], rep, axis=1)
        v = jnp.repeat(v_cache[:, :, Sk - W:, :], rep, axis=1)
        scores = jnp.einsum("bhqd,bhkd->bhqk", q, k) * (Dh ** -0.5)
        p = _softmax(scores, axis=-1)
        o = jnp.einsum("bhqk,bhkd->bhqd", p, v)
        return (lambda x, *d: x.transpose(*d))(o, 0, 2, 1, 3).reshape(B, Sq, Hq * Dh) @ wo

    def _B_ref(x, k_cache, v_cache, wq, wo):
        B, Sq, D = x.shape
        Hq, Dh = 32, 128
        Hkv, Sk = k_cache.shape[1], k_cache.shape[2]
        W = min(4096, max(256, Sk // 4))
        rep = Hq // Hkv
        q = (lambda x, *d: x.transpose(*d))((x @ wq).reshape(B, Sq, Hq, Dh), 0, 2, 1, 3)
        k = jnp.repeat(k_cache[:, :, Sk - W:, :], rep, axis=1)
        v = jnp.repeat(v_cache[:, :, Sk - W:, :], rep, axis=1)
        scores = jnp.einsum("bhqd,bhkd->bhqk", q, k) * (Dh ** -0.5)
        p = _softmax(scores, axis=-1)
        o = jnp.einsum("bhqk,bhkd->bhqd", p, v)
        return (lambda x, *d: x.transpose(*d))(o, 0, 2, 1, 3).reshape(B, Sq, Hq * Dh) @ wo

    a = _A_ref(A_x, A_k_cache, A_v_cache, A_wq, A_wo)
    b = _B_ref(B_x, B_k_cache, B_v_cache, B_wq, B_wo)
    return jnp.concatenate([a, b], axis=-1)
```

```python
import jax, jax.numpy as jnp
from jax import lax
import jax.experimental.pallas as pl
import jax.experimental.pallas.tpu as pltpu

B, D, HQ, HKV, SK, DH = 4, 576, 32, 16, 8192, 128
W = 2048
N = HQ * DH
SCALE = DH ** -0.5

def make(HB=4, RPD=32, NC=4, LA=3, QG=9, QC=256, OG=4, OC=512, abl=''):
    NHB = HKV // HB
    UPP = NHB * B
    NU = 2 * UPP
    CH = W // NC
    assert LA < NC
    QR = D // QG
    OR = D // OG
    HC = 2 * HB * DH
    NQ = QR // 8
    OB = 16
    NO = OR // OB

    def kern(ax, ak, av, awq, awo, bx, bk, bv, bwq, bwo, o_ref,
             xbuf, wqbuf, wobuf, kvbuf, q_sc, lhs_sc, out_sc,
             xsem, wqsem, wosem, kvsem):
        xs = (ax, bx); ks = (ak, bk); vs = (av, bv); wqs = (awq, bwq); wos = (awo, bwo)

        def issue_kv(p, u, c):
            hb = u // B
            b = u % B
            for r0 in range(0, CH, RPD):
                for a, src in enumerate((ks[p], vs[p])):
                    pltpu.make_async_copy(
                        src.at[b, pl.ds(hb * HB, HB), pl.ds(SK - W + c * CH + r0, RPD), :],
                        kvbuf.at[c, a, :, pl.ds(r0, RPD), :], kvsem.at[c]).start(priority=a)

        def issue_wq(g):
            rr = g * 8
            for c0 in range(0, N, QC):
                for p in range(2):
                    pltpu.make_async_copy(
                        wqs[p].at[:, pl.ds(rr, 8), pl.ds(c0, QC)],
                        wqbuf.at[p, c0 // HC, :, pl.ds(rr, 8), pl.ds(c0 % HC, QC)], wqsem.at[g]).start(priority=p)

        def wait_wq(g):
            v = wqbuf.at[:, :, :, pl.ds(g * 8, 8), :]
            pltpu.make_async_copy(v, v, wqsem.at[g]).wait()

        def issue_wo(g):
            for rr in range(g * OB, (g + 1) * OB, 8):
                for c0 in range(0, N, OC):
                    for p in range(2):
                        pltpu.make_async_copy(
                            wos[p].at[:, pl.ds(rr, 8), pl.ds(c0, OC)],
                            wobuf.at[p, :, pl.ds(rr, 8), pl.ds(c0, OC)], wosem.at[g]).start(priority=p)

        def wait_wo(g):
            v = wobuf.at[:, :, pl.ds(g * OB, OB), :]
            pltpu.make_async_copy(v, v, wosem.at[g]).wait()

        for g in range(LA):
            issue_wq(g)
        xc = [pltpu.make_async_copy(xs[p], xbuf.at[p], xsem.at[p]) for p in range(2)]
        for c in xc: c.start()
        lhs_sc[...] = jnp.zeros_like(lhs_sc)
        for g in range(NQ):
            wait_wq(g)
            if g + LA < NQ:
                issue_wq(g + LA)
            else:
                issue_kv(0, 0, g + LA - NQ)
        for c in xc: c.wait()
        row = lax.broadcasted_iota(jnp.int32, (8, DH), 0)

        def unit(u, carry):
            p = u // UPP
            ul = u % UPP
            hb = ul // B
            b = ul % B
            @pl.when(b == 0)
            def _():
                x = xbuf[p].astype(jnp.float32)
                x8 = jnp.concatenate([x, x], axis=0).astype(jnp.bfloat16)
                wq = wqbuf[p, hb].reshape(D, HC)
                q = jnp.dot(x8, wq, preferred_element_type=jnp.float32)
                for hh in range(HB):
                    q_sc[hh] = jnp.where(row < B, q[:, (2*hh)*DH:(2*hh+1)*DH], q[:, (2*hh+1)*DH:(2*hh+2)*DH]).astype(jnp.bfloat16)
            ms = [None] * HB; ls = [None] * HB; accs = [None] * HB
            for c in range(NC):
                pltpu.make_async_copy(kvbuf.at[c], kvbuf.at[c], kvsem.at[c]).wait()
                cn = c + LA
                if cn < NC:
                    @pl.when(u < UPP)
                    def _():
                        issue_kv(0, u, cn)
                    @pl.when(u >= UPP)
                    def _():
                        issue_kv(1, u - UPP, cn)
                else:
                    cn -= NC
                    @pl.when(u + 1 < UPP)
                    def _():
                        issue_kv(0, u + 1, cn)
                    @pl.when((u + 1 >= UPP) & (u + 1 < NU))
                    def _():
                        issue_kv(1, u + 1 - UPP, cn)
                    @pl.when(u + 1 == NU)
                    def _():
                        issue_wo(cn)
                for hh in range(0 if 'a' in abl else HB):
                    qh = q_sc[hh]
                    sc = lax.dot_general(qh, kvbuf[c, 0, hh], (((1,), (1,)), ((), ())), preferred_element_type=jnp.float32)
                    mc = jnp.max(sc, axis=-1, keepdims=True)
                    if c == 0:
                        m = mc
                    else:
                        m = jnp.maximum(ms[hh], mc)
                        alpha = jnp.exp((ms[hh] - m) * SCALE)
                    e = jnp.exp((sc - m) * SCALE)
                    lp = e[:, 0:DH]
                    for j in range(1, CH // DH):
                        lp = lp + e[:, j*DH:(j+1)*DH]
                    pv = jnp.dot(e.astype(jnp.bfloat16), kvbuf[c, 1, hh], preferred_element_type=jnp.float32)
                    if c == 0:
                        ls[hh] = lp; accs[hh] = pv
                    else:
                        ls[hh] = ls[hh] * alpha + lp
                        accs[hh] = accs[hh] * alpha + pv
                    ms[hh] = m
            for hh in range(0 if 'a' in abl else HB):
                h = hb * HB + hh
                o = accs[hh] / jnp.sum(ls[hh], axis=-1, keepdims=True)
                pltpu.store(lhs_sc.at[p, 2*h], o, mask=row == b)
                pltpu.store(lhs_sc.at[p, 2*h+1], o, mask=row == b + B)
            return carry
        lax.fori_loop(0, NU, unit, 0)

        lhs = [jnp.concatenate([lhs_sc[p, j] for j in range(HQ)], axis=1).astype(jnp.bfloat16) for p in range(2)]
        for g in range(NO):
            wait_wo(g)
            if g + LA < NO:
                issue_wo(g + LA)
            r0 = g * OB
            for p in range(2):
                w = wobuf[p, :, r0:r0+OB, :].reshape(OG * OB, N)
                r = lax.dot_general(lhs[p], w, (((1,), (1,)), ((), ())), preferred_element_type=jnp.float32)
                r4 = r[0:B] + r[B:2*B]
                for j in range(OG):
                    n0 = p * D + j * OR + r0
                    out_sc[:, n0:n0+OB] = r4[:, j*OB:(j+1)*OB]
        o_ref[...] = out_sc[...].astype(o_ref.dtype)

    @jax.jit
    def fn(A_x, A_k_cache, A_v_cache, A_wq, A_wo, B_x, B_k_cache, B_v_cache, B_wq, B_wo):
        hbm = pl.BlockSpec(memory_space=pltpu.HBM)
        bf = jnp.bfloat16
        out = pl.pallas_call(
            kern,
            in_specs=[hbm]*10,
            out_specs=pl.BlockSpec(memory_space=pltpu.VMEM),
            out_shape=jax.ShapeDtypeStruct((B, 2*D), bf),
            scratch_shapes=[
                pltpu.VMEM((2, B, D), bf),
                pltpu.VMEM((2, NHB, QG, QR, HC), bf),
                pltpu.VMEM((2, OG, OR, N), bf),
                pltpu.VMEM((NC, 2, HB, CH, DH), bf),
                pltpu.VMEM((HB, 8, DH), bf),
                pltpu.VMEM((2, HQ, 8, DH), jnp.float32),
                pltpu.VMEM((B, 2*D), jnp.float32),
                pltpu.SemaphoreType.DMA((2,)),
                pltpu.SemaphoreType.DMA((NQ,)),
                pltpu.SemaphoreType.DMA((NO,)),
                pltpu.SemaphoreType.DMA((NC,)),
            ],
            compiler_params=pltpu.CompilerParams(vmem_limit_bytes=100*1024*1024),
        )(A_x.reshape(B, D), A_k_cache, A_v_cache, A_wq.reshape(QG, QR, N), A_wo.T.reshape(OG, OR, N),
          B_x.reshape(B, D), B_k_cache, B_v_cache, B_wq.reshape(QG, QR, N), B_wo.T.reshape(OG, OR, N))
        return out.reshape(B, 1, 2*D)
    return fn


pallas_concat_heads__sliding_block_cached__sliding_block_cached__decode_kernel = make()
```

```python
import jax, jax.numpy as jnp
from jax import lax
import jax.experimental.pallas as pl
import jax.experimental.pallas.tpu as pltpu

B, D, HQ, HKV, SK, DH = 4, 576, 32, 16, 8192, 128
W = 2048
N = HQ * DH
SCALE = DH ** -0.5
NT = (((1,), (1,)), ((), ()))

def make(HB=8, RPD=16, NC=8, LA=3, SUBS=(2, 2), QG=9, QC=256, OG=4, OC=512, abl='', semchk=False):
    NHB = HKV // HB
    UPP = NHB * B
    NU = 2 * UPP
    CH = W // NC
    NS = LA + 1
    assert NC % NS == 0
    QR = D // QG
    OR = D // OG
    HC = 2 * HB * DH
    NQ = QR // 8
    OB = 16
    NO = OR // OB
    nsub = [1] * (NO - len(SUBS)) + list(SUBS)
    sem_base = [sum(nsub[:g]) for g in range(NO)]
    NSEM = sum(nsub)
    MAXS = max(nsub)
    rords = []
    for p in range(2):
        allr = [g * OB for g in range(NO)]
        good = [r for r in allr if (p * D + r) % 128 == 0][-1]
        rords.append([r for r in allr if r != good] + [good])

    def kern(ax, ak, av, awq, awo, bx, bk, bv, bwq, bwo, o_ref,
             xbuf, wqbuf, wobuf, kvbuf, q_sc, lhs_sc, out_sc, res_sc,
             xsem, wqsem, wosem, kvsem):
        xs = (ax, bx); ks = (ak, bk); vs = (av, bv); wqs = (awq, bwq); wos = (awo, bwo)

        def issue_kv(p, u, c):
            hb = u // B
            b = u % B
            slot = c % NS
            for r0 in range(0, CH, RPD):
                for a, src in enumerate((ks[p], vs[p])):
                    pltpu.make_async_copy(
                        src.at[b, pl.ds(hb * HB, HB), pl.ds(SK - W + c * CH + r0, RPD), :],
                        kvbuf.at[slot, a, :, pl.ds(r0, RPD), :], kvsem.at[slot]).start(priority=a)

        def issue_wq(g):
            rr = g * 8
            for c0 in range(0, N, QC):
                for p in range(2):
                    pltpu.make_async_copy(
                        wqs[p].at[:, pl.ds(rr, 8), pl.ds(c0, QC)],
                        wqbuf.at[p, c0 // HC, :, pl.ds(rr, 8), pl.ds(c0 % HC, QC)], wqsem.at[g]).start(priority=p)

        def wait_wq(g):
            v = wqbuf.at[:, :, :, pl.ds(g * 8, 8), :]
            pltpu.make_async_copy(v, v, wqsem.at[g]).wait()

        def issue_wo(g):
            subc = N // nsub[g]
            for s in range(nsub[g]):
                for rr in range(0, OB, 8):
                    for c0 in range(s * subc, (s + 1) * subc, OC):
                        for p in range(2):
                            pltpu.make_async_copy(
                                wos[p].at[:, pl.ds(rords[p][g] + rr, 8), pl.ds(c0, OC)],
                                wobuf.at[g, p, :, pl.ds(rr, 8), pl.ds(c0, OC)], wosem.at[sem_base[g] + s]).start(priority=p)

        for g in range(LA):
            issue_wq(g)
        xc = [pltpu.make_async_copy(xs[p], xbuf.at[p], xsem.at[p]) for p in range(2)]
        for p, c in enumerate(xc): c.start(priority=p)
        lhs_sc[...] = jnp.zeros_like(lhs_sc)
        if abl:
            out_sc[...] = jnp.zeros_like(out_sc)
            q_sc[...] = jnp.zeros_like(q_sc)
        for g in range(NQ):
            wait_wq(g)
            if g + LA < NQ:
                issue_wq(g + LA)
            else:
                issue_kv(0, 0, g + LA - NQ)
        for c in xc: c.wait()
        row = lax.broadcasted_iota(jnp.int32, (8, DH), 0)
        HH = range(0 if 'a' in abl else HB)

        def unit(u, carry):
            p = u // UPP
            ul = u % UPP
            hb = ul // B
            b = ul % B
            if 'q' not in abl:
                @pl.when(b == 0)
                def _():
                    x = xbuf[p].astype(jnp.float32)
                    x8 = jnp.concatenate([x, x], axis=0).astype(jnp.bfloat16)
                    wq = wqbuf[p, hb].reshape(D, HC)
                    q = jnp.dot(x8, wq, preferred_element_type=jnp.float32)
                    for hh in range(HB):
                        q_sc[hh] = jnp.where(row < B, q[:, (2*hh)*DH:(2*hh+1)*DH], q[:, (2*hh+1)*DH:(2*hh+2)*DH]).astype(jnp.bfloat16)
            ms = [None] * HB; ls = [None] * HB; accs = [None] * HB
            for c in range(NC):
                slot = c % NS
                pltpu.make_async_copy(kvbuf.at[slot], kvbuf.at[slot], kvsem.at[slot]).wait()
                cn = c + LA
                if cn < NC:
                    @pl.when(u < UPP)
                    def _():
                        issue_kv(0, u, cn)
                    @pl.when(u >= UPP)
                    def _():
                        issue_kv(1, u - UPP, cn)
                else:
                    cn -= NC
                    @pl.when(u + 1 < UPP)
                    def _():
                        issue_kv(0, u + 1, cn)
                    @pl.when((u + 1 >= UPP) & (u + 1 < NU))
                    def _():
                        issue_kv(1, u + 1 - UPP, cn)
                    @pl.when(u + 1 == NU)
                    def _():
                        issue_wo(cn)
                scs = [lax.dot_general(q_sc[hh], kvbuf[slot, 0, hh], NT, preferred_element_type=jnp.float32) for hh in HH]
                es = []; alphas = []
                for hh in HH:
                    sc = scs[hh]
                    mc = jnp.max(sc, axis=-1, keepdims=True)
                    if c == 0:
                        m = mc
                    else:
                        m = jnp.maximum(ms[hh], mc)
                        alphas.append(jnp.exp((ms[hh] - m) * SCALE))
                    e = jnp.exp((sc - m) * SCALE)
                    lp = e[:, 0:DH]
                    for j in range(1, CH // DH):
                        lp = lp + e[:, j*DH:(j+1)*DH]
                    ls[hh] = lp if c == 0 else ls[hh] * alphas[hh] + lp
                    ms[hh] = m
                    es.append(e.astype(jnp.bfloat16))
                for hh in HH:
                    pv = jnp.dot(es[hh], kvbuf[slot, 1, hh], preferred_element_type=jnp.float32)
                    accs[hh] = pv if c == 0 else accs[hh] * alphas[hh] + pv
            for hh in HH:
                h = hb * HB + hh
                o = accs[hh] / jnp.sum(ls[hh], axis=-1, keepdims=True)
                pltpu.store(lhs_sc.at[p, 2*h], o, mask=row == b)
                pltpu.store(lhs_sc.at[p, 2*h+1], o, mask=row == b + B)
            return carry
        lax.fori_loop(0, NU, unit, 0)

        lhs = [jnp.concatenate([lhs_sc[p, j] for j in range(HQ)], axis=1).astype(jnp.bfloat16) for p in range(2)]
        PP = range(0 if 'o' in abl else 2)
        def emit(g):
            for p in PP:
                r = res_sc[p, g, 0]
                for s in range(1, nsub[g]):
                    r = r + res_sc[p, g, s]
                r4 = r[0:B] + r[B:2*B]
                for j in range(OG):
                    n0 = p * D + j * OR + rords[p][g]
                    out_sc[:, n0:n0+OB] = r4[:, j*OB:(j+1)*OB]
        for g in range(NO):
            subc = N // nsub[g]
            for s in range(nsub[g]):
                v = wobuf.at[g, :, :, :, pl.ds(s * subc, subc)]
                pltpu.make_async_copy(v, v, wosem.at[sem_base[g] + s]).wait()
                if s == nsub[g] - 1 and g + LA < NO:
                    issue_wo(g + LA)
                if s == 0 and g > 0:
                    emit(g - 1)
                for p in PP:
                    w = wobuf[g, p, :, :, s*subc:(s+1)*subc].reshape(OG * OB, subc)
                    res_sc[p, g, s] = lax.dot_general(lhs[p][:, s*subc:(s+1)*subc], w, NT, preferred_element_type=jnp.float32)
        emit(NO - 1)
        o_ref[...] = out_sc[...].astype(o_ref.dtype)

    @jax.jit
    def fn(A_x, A_k_cache, A_v_cache, A_wq, A_wo, B_x, B_k_cache, B_v_cache, B_wq, B_wo):
        hbm = pl.BlockSpec(memory_space=pltpu.HBM)
        bf = jnp.bfloat16
        out = pl.pallas_call(
            kern,
            in_specs=[hbm]*10,
            out_specs=pl.BlockSpec(memory_space=pltpu.VMEM),
            out_shape=jax.ShapeDtypeStruct((B, 2*D), bf),
            scratch_shapes=[
                pltpu.VMEM((2, B, D), bf),
                pltpu.VMEM((2, NHB, QG, QR, HC), bf),
                pltpu.VMEM((NO, 2, OG, OB, N), bf),
                pltpu.VMEM((NS, 2, HB, CH, DH), bf),
                pltpu.VMEM((HB, 8, DH), bf),
                pltpu.VMEM((2, HQ, 8, DH), jnp.float32),
                pltpu.VMEM((B, 2*D), jnp.float32),
                pltpu.VMEM((2, NO, MAXS, 8, OG * OB), jnp.float32),
                pltpu.SemaphoreType.DMA((2,)),
                pltpu.SemaphoreType.DMA((NQ,)),
                pltpu.SemaphoreType.DMA((NSEM,)),
                pltpu.SemaphoreType.DMA((NS,)),
            ],
            compiler_params=pltpu.CompilerParams(vmem_limit_bytes=100*1024*1024, disable_bounds_checks=True, disable_semaphore_checks=not semchk),
        )(A_x.reshape(B, D), A_k_cache, A_v_cache, A_wq.reshape(QG, QR, N), A_wo.T.reshape(OG, OR, N),
          B_x.reshape(B, D), B_k_cache, B_v_cache, B_wq.reshape(QG, QR, N), B_wo.T.reshape(OG, OR, N))
        return out.reshape(B, 1, 2*D)
    return fn


pallas_concat_heads__sliding_block_cached__sliding_block_cached__decode_kernel = make()
```

```python
import jax, jax.numpy as jnp
from jax import lax
import jax.experimental.pallas as pl
import jax.experimental.pallas.tpu as pltpu

B, D, HQ, HKV, SK, DH = 4, 576, 32, 16, 8192, 128
W = 2048
N = HQ * DH
SCALE = DH ** -0.5
NT = (((1,), (1,)), ((), ()))

def make(HB=8, RPD=16, NC=8, LA=3, WG=9, WC=128, WS=2, OWC=256, OWS=2, OLA=6, SKEW=2, LASTS=(), abl=''):
    NHB = HKV // HB
    UPP = NHB * B
    NU = 2 * UPP
    CH = W // NC
    NS = LA + 1
    assert NC % NS == 0
    WR = D // WG
    HC = 2 * HB * DH
    NBAND = WR // 8
    SC = N // WS
    NW = NBAND * WS
    OSC = N // OWS
    ONW = NBAND * OWS
    assert OLA % LA == 0
    OPER = OLA // LA

    lastcuts = [0]
    for z in (LASTS or (OSC,)):
        lastcuts.append(lastcuts[-1] + z)
    assert lastcuts[-1] == OSC
    def osem(g, p, c):
        if g == ONW - 1 and p == 1:
            k = max(i for i in range(len(lastcuts) - 1) if lastcuts[i] <= c)
            return 2 * g + p + k
        return 2 * g + p

    def kern(ax, ak, av, awq, awo, bx, bk, bv, bwq, bwo, o_ref,
             xbuf, wqbuf, wobuf, kvbuf, q_sc, lhs_sc, out_sc, res_sc,
             xsem, wqsem, wosem, kvsem):
        xs = (ax, bx); ks = (ak, bk); vs = (av, bv); wqs = (awq, bwq); wos = (awo, bwo)

        def issue_kv(p, u, c):
            hb = u % NHB
            b = u // NHB
            slot = c % NS
            for r0 in range(0, CH, RPD):
                for a, src in enumerate((ks[p], vs[p])):
                    pltpu.make_async_copy(
                        src.at[b, pl.ds(hb * HB, HB), pl.ds(SK - W + c * CH + r0, RPD), :],
                        kvbuf.at[slot, a, :, pl.ds(r0, RPD), :], kvsem.at[slot]).start(priority=a)

        def issue_wq(g):
            rr = (g // WS) * 8
            s = g % WS
            for c0 in range(s * SC, (s + 1) * SC, WC):
                for p in range(2):
                    pltpu.make_async_copy(
                        wqs[p].at[:, pl.ds(rr, 8), pl.ds(c0, WC)],
                        wqbuf.at[p, c0 // HC, :, pl.ds(rr, 8), pl.ds(c0 % HC, WC)], wqsem.at[g]).start(priority=p)

        def wait_wq(g):
            rr = (g // WS) * 8
            s = g % WS
            if SC >= HC:
                v = wqbuf.at[:, pl.ds(s * SC // HC, SC // HC), :, pl.ds(rr, 8), :]
            else:
                v = wqbuf.at[:, s * SC // HC, :, pl.ds(rr, 8), pl.ds((s * SC) % HC, SC)]
            pltpu.make_async_copy(v, v, wqsem.at[g]).wait()

        def issue_wo(g):
            band = g // OWS
            s = g % OWS
            for c0 in range(s * OSC, (s + 1) * OSC, OWC):
                for p in range(2):
                    pltpu.make_async_copy(
                        wos[p].at[:, pl.ds(band * 8, 8), pl.ds(c0, OWC)],
                        wobuf.at[g, p, :, :, pl.ds(c0 - s * OSC, OWC)], wosem.at[osem(g, p, c0 - s * OSC)]).start(priority=p)

        for g in range(LA):
            issue_wq(g)
        xc = [pltpu.make_async_copy(xs[p], xbuf.at[p], xsem.at[p]) for p in range(2)]
        for p, c in enumerate(xc): c.start(priority=p)
        lhs_sc[...] = jnp.zeros_like(lhs_sc)
        if abl:
            out_sc[...] = jnp.zeros_like(out_sc)
            q_sc[...] = jnp.zeros_like(q_sc)
        for g in range(NW):
            wait_wq(g)
            if g + LA < NW:
                issue_wq(g + LA)
            else:
                issue_kv(0, 0, g + LA - NW)
        for c in xc: c.wait()
        row = lax.broadcasted_iota(jnp.int32, (8, DH), 0)
        HH = range(0 if 'a' in abl else HB)

        def unit(u, carry):
            p = u // UPP
            ul = u % UPP
            hb = ul % NHB
            b = ul // NHB
            if 'q' not in abl:
                @pl.when(b == 0)
                def _():
                    x = xbuf[p].astype(jnp.float32)
                    x8 = jnp.concatenate([x, x], axis=0).astype(jnp.bfloat16)
                    wq = wqbuf[p, hb].reshape(D, HC)
                    q = jnp.dot(x8, wq, preferred_element_type=jnp.float32)
                    for hh in range(HB):
                        q_sc[hb, hh] = jnp.where(row < B, q[:, (2*hh)*DH:(2*hh+1)*DH], q[:, (2*hh+1)*DH:(2*hh+2)*DH]).astype(jnp.bfloat16)
            ms = [None] * HB; ls = [None] * HB; accs = [None] * HB
            for c in range(NC):
                slot = c % NS
                pltpu.make_async_copy(kvbuf.at[slot], kvbuf.at[slot], kvsem.at[slot]).wait()
                cn = c + LA
                if cn < NC:
                    @pl.when(u < UPP)
                    def _():
                        issue_kv(0, u, cn)
                    @pl.when(u >= UPP)
                    def _():
                        issue_kv(1, u - UPP, cn)
                else:
                    cn -= NC
                    @pl.when(u + 1 < UPP)
                    def _():
                        issue_kv(0, u + 1, cn)
                    @pl.when((u + 1 >= UPP) & (u + 1 < NU))
                    def _():
                        issue_kv(1, u + 1 - UPP, cn)
                    @pl.when(u + 1 == NU)
                    def _():
                        for gg in range(cn * OPER, (cn + 1) * OPER):
                            issue_wo(gg)
                scs = [lax.dot_general(q_sc[hb, hh], kvbuf[slot, 0, hh], NT, preferred_element_type=jnp.float32) for hh in HH]
                es = []; alphas = []
                for hh in HH:
                    sc = scs[hh]
                    mc = jnp.max(sc, axis=-1, keepdims=True)
                    if c == 0:
                        m = mc
                    else:
                        m = jnp.maximum(ms[hh], mc)
                        alphas.append(jnp.exp((ms[hh] - m) * SCALE))
                    e = jnp.exp((sc - m) * SCALE)
                    lp = e[:, 0:DH]
                    for j in range(1, CH // DH):
                        lp = lp + e[:, j*DH:(j+1)*DH]
                    ls[hh] = lp if c == 0 else ls[hh] * alphas[hh] + lp
                    ms[hh] = m
                    es.append(e.astype(jnp.bfloat16))
                for hh in HH:
                    pv = jnp.dot(es[hh], kvbuf[slot, 1, hh], preferred_element_type=jnp.float32)
                    accs[hh] = pv if c == 0 else accs[hh] * alphas[hh] + pv
            for hh in HH:
                h = hb * HB + hh
                o = accs[hh] / jnp.sum(ls[hh], axis=-1, keepdims=True)
                pltpu.store(lhs_sc.at[p, 2*h], o, mask=row == b)
                pltpu.store(lhs_sc.at[p, 2*h+1], o, mask=row == b + B)
            return carry
        lax.fori_loop(0, NU, unit, 0)

        lhs = [jnp.concatenate([lhs_sc[p, j] for j in range(HQ)], axis=1).astype(jnp.bfloat16) for p in range(2)]
        PP = range(0 if 'o' in abl else 2)
        nlast = len(lastcuts) - 1
        def emit(p, band):
            r = res_sc[p, band * OWS]
            for s in range(1, OWS + (nlast - 1 if (p == 1 and band == NBAND - 1) else 0)):
                r = r + res_sc[p, band * OWS + s]
            r4 = r[0:B] + r[B:2*B]
            for j in range(WG):
                n0 = p * D + j * WR + band * 8
                out_sc[:, n0:n0+8] = r4[:, j*8:(j+1)*8]
        order = [(0, g) for g in range(min(SKEW, ONW))]
        for g in range(ONW):
            if g + SKEW < ONW:
                order.append((0, g + SKEW)) if SKEW == 0 else None
            order.append((1, g))
            if SKEW > 0 and g + SKEW < ONW:
                order.append((0, g + SKEW))
        pending = []
        for (p, g) in order:
            s = g % OWS
            cuts = lastcuts if (p == 1 and g == ONW - 1) else [0, OSC]
            for k in range(len(cuts) - 1):
                c0, c1 = cuts[k], cuts[k + 1]
                v = wobuf.at[g, p, :, :, pl.ds(c0, c1 - c0)]
                pltpu.make_async_copy(v, v, wosem.at[osem(g, p, c0)]).wait()
                if p == 1 and g + OLA < ONW:
                    issue_wo(g + OLA)
                if 'o' in abl:
                    continue
                for e in pending:
                    emit(*e)
                pending = []
                w = wobuf[g, p, :, :, c0:c1].reshape(WG * 8, c1 - c0)
                res_sc[p, g + k] = lax.dot_general(lhs[p][:, s*OSC+c0:s*OSC+c1], w, NT, preferred_element_type=jnp.float32)
            if s == OWS - 1:
                pending.append((p, g // OWS))
        if 'o' not in abl:
            for e in pending:
                emit(*e)
        o_ref[...] = out_sc[...].astype(o_ref.dtype)

    @jax.jit
    def fn(A_x, A_k_cache, A_v_cache, A_wq, A_wo, B_x, B_k_cache, B_v_cache, B_wq, B_wo):
        hbm = pl.BlockSpec(memory_space=pltpu.HBM)
        bf = jnp.bfloat16
        out = pl.pallas_call(
            kern,
            in_specs=[hbm]*10,
            out_specs=pl.BlockSpec(memory_space=pltpu.VMEM),
            out_shape=jax.ShapeDtypeStruct((B, 2*D), bf),
            scratch_shapes=[
                pltpu.VMEM((2, B, D), bf),
                pltpu.VMEM((2, NHB, WG, WR, HC), bf),
                pltpu.VMEM((ONW, 2, WG, 8, OSC), bf),
                pltpu.VMEM((NS, 2, HB, CH, DH), bf),
                pltpu.VMEM((NHB, HB, 8, DH), bf),
                pltpu.VMEM((2, HQ, 8, DH), jnp.float32),
                pltpu.VMEM((B, 2*D), jnp.float32),
                pltpu.VMEM((2, ONW + 4, 8, WG * 8), jnp.float32),
                pltpu.SemaphoreType.DMA((2,)),
                pltpu.SemaphoreType.DMA((NW,)),
                pltpu.SemaphoreType.DMA((2 * ONW + len(LASTS),)),
                pltpu.SemaphoreType.DMA((NS,)),
            ],
            compiler_params=pltpu.CompilerParams(vmem_limit_bytes=100*1024*1024, disable_bounds_checks=True, disable_semaphore_checks=True),
        )(A_x.reshape(B, D), A_k_cache, A_v_cache, A_wq.reshape(WG, WR, N), A_wo.T.reshape(WG, WR, N),
          B_x.reshape(B, D), B_k_cache, B_v_cache, B_wq.reshape(WG, WR, N), B_wo.T.reshape(WG, WR, N))
        return out.reshape(B, 1, 2*D)
    return fn


pallas_concat_heads__sliding_block_cached__sliding_block_cached__decode_kernel = make(SKEW=3, LASTS=(1024, 1024))
```

```python
import jax
import jax.numpy as jnp
from jax import lax
import jax.experimental.pallas as pl
import jax.experimental.pallas.tpu as pltpu

_NT = (((1,), (1,)), ((), ()))

HQ = 32
DH = 128
HB = 8
RPD = 16
NC = 8
LA = 3
NS = LA + 1
WG = 9
QC = 128
QS = 2
OC = 256
OS = 2
OLA = 6
SKEW = 3
LAST_SPLIT = 2


@jax.jit
def pallas_concat_heads__sliding_block_cached__sliding_block_cached__decode_kernel(
    A_x: jax.Array,
    A_k_cache: jax.Array,
    A_v_cache: jax.Array,
    A_wq: jax.Array,
    A_wo: jax.Array,
    B_x: jax.Array,
    B_k_cache: jax.Array,
    B_v_cache: jax.Array,
    B_wq: jax.Array,
    B_wo: jax.Array,
):
    B, SQ, D = A_x.shape
    _, HKV, SK, _ = A_k_cache.shape
    N = HQ * DH
    W = min(4096, max(256, SK // 4))
    assert SQ == 1 and HQ == 2 * HKV and 2 * B == 8
    scale = DH ** -0.5

    NHB = HKV // HB
    UPP = NHB * B
    NU = 2 * UPP
    CH = W // NC
    HC = 2 * HB * DH
    WR = D // WG
    NBAND = WR // 8
    QSC = N // QS
    NQ = NBAND * QS
    OSC = N // OS
    NO = NBAND * OS
    OPER = OLA // LA
    LASTC = OSC // LAST_SPLIT
    assert NC % NS == 0 and OLA % LA == 0 and QSC == HC and SKEW < OLA

    def wo_sem(g, p, col):
        extra = col // LASTC if (g == NO - 1 and p == 1) else 0
        return 2 * g + p + extra

    def kernel(ax, ak, av, awq, awo, bx, bk, bv, bwq, bwo, o_ref,
               xbuf, wqbuf, wobuf, kvbuf, q_sc, lhs_sc, out_sc, res_sc,
               xsem, wqsem, wosem, kvsem):
        xs, ks, vs, wqs, wos = (ax, bx), (ak, bk), (av, bv), (awq, bwq), (awo, bwo)

        def wait_all(view, sem):
            pltpu.make_async_copy(view, view, sem).wait()

        def issue_kv(p, u, c):
            hb = u % NHB
            b = u // NHB
            slot = c % NS
            for r0 in range(0, CH, RPD):
                for a, src in enumerate((ks[p], vs[p])):
                    pltpu.make_async_copy(
                        src.at[b, pl.ds(hb * HB, HB), pl.ds(SK - W + c * CH + r0, RPD), :],
                        kvbuf.at[slot, a, :, pl.ds(r0, RPD), :],
                        kvsem.at[slot],
                    ).start(priority=a)

        def issue_wq(g):
            rr, s = (g // QS) * 8, g % QS
            for c0 in range(0, QSC, QC):
                for p in range(2):
                    pltpu.make_async_copy(
                        wqs[p].at[:, pl.ds(rr, 8), pl.ds(s * QSC + c0, QC)],
                        wqbuf.at[p, s, :, pl.ds(rr, 8), pl.ds(c0, QC)],
                        wqsem.at[g],
                    ).start(priority=p)

        def issue_wo(g):
            band, s = g // OS, g % OS
            for c0 in range(0, OSC, OC):
                for p in range(2):
                    pltpu.make_async_copy(
                        wos[p].at[:, pl.ds(band * 8, 8), pl.ds(s * OSC + c0, OC)],
                        wobuf.at[g, p, :, :, pl.ds(c0, OC)],
                        wosem.at[wo_sem(g, p, c0)],
                    ).start(priority=p)

        for g in range(LA):
            issue_wq(g)
        xcopies = [pltpu.make_async_copy(xs[p], xbuf.at[p], xsem.at[p]) for p in range(2)]
        for p in range(2):
            xcopies[p].start(priority=p)
        lhs_sc[...] = jnp.zeros_like(lhs_sc)
        for g in range(NQ):
            wait_all(wqbuf.at[:, g % QS, :, pl.ds((g // QS) * 8, 8), :], wqsem.at[g])
            if g + LA < NQ:
                issue_wq(g + LA)
            else:
                issue_kv(0, 0, g + LA - NQ)
        for p in range(2):
            xcopies[p].wait()

        row = lax.broadcasted_iota(jnp.int32, (8, DH), 0)

        def unit(u, carry):
            p = u // UPP
            ul = u % UPP
            hb = ul % NHB
            b = ul // NHB

            @pl.when(b == 0)
            def _():
                x = xbuf[p].astype(jnp.float32)
                x8 = jnp.concatenate([x, x], axis=0).astype(jnp.bfloat16)
                wq = wqbuf[p, hb].reshape(D, HC)
                q = jnp.dot(x8, wq, preferred_element_type=jnp.float32)
                for hh in range(HB):
                    q0 = q[:, (2 * hh) * DH:(2 * hh + 1) * DH]
                    q1 = q[:, (2 * hh + 1) * DH:(2 * hh + 2) * DH]
                    q_sc[hb, hh] = jnp.where(row < B, q0, q1).astype(jnp.bfloat16)

            ms, ls, accs = [None] * HB, [None] * HB, [None] * HB
            for c in range(NC):
                slot = c % NS
                wait_all(kvbuf.at[slot], kvsem.at[slot])

                cn = c + LA
                if cn < NC:
                    @pl.when(u < UPP)
                    def _():
                        issue_kv(0, u, cn)

                    @pl.when(u >= UPP)
                    def _():
                        issue_kv(1, u - UPP, cn)
                else:
                    cn -= NC

                    @pl.when(u + 1 < UPP)
                    def _():
                        issue_kv(0, u + 1, cn)

                    @pl.when((u + 1 >= UPP) & (u + 1 < NU))
                    def _():
                        issue_kv(1, u + 1 - UPP, cn)

                    @pl.when(u + 1 == NU)
                    def _():
                        for g in range(cn * OPER, (cn + 1) * OPER):
                            issue_wo(g)

                scores = [
                    lax.dot_general(q_sc[hb, hh], kvbuf[slot, 0, hh], _NT,
                                    preferred_element_type=jnp.float32)
                    for hh in range(HB)
                ]
                probs, alphas = [], []
                for hh in range(HB):
                    sc = scores[hh]
                    m = jnp.max(sc, axis=-1, keepdims=True)
                    if c > 0:
                        m = jnp.maximum(ms[hh], m)
                        alphas.append(jnp.exp((ms[hh] - m) * scale))
                    e = jnp.exp((sc - m) * scale)
                    lp = e[:, 0:DH]
                    for j in range(1, CH // DH):
                        lp = lp + e[:, j * DH:(j + 1) * DH]
                    ls[hh] = lp if c == 0 else ls[hh] * alphas[hh] + lp
                    ms[hh] = m
                    probs.append(e.astype(jnp.bfloat16))
                for hh in range(HB):
                    pv = jnp.dot(probs[hh], kvbuf[slot, 1, hh],
                                 preferred_element_type=jnp.float32)
                    accs[hh] = pv if c == 0 else accs[hh] * alphas[hh] + pv

            for hh in range(HB):
                h = hb * HB + hh
                o = accs[hh] / jnp.sum(ls[hh], axis=-1, keepdims=True)
                pltpu.store(lhs_sc.at[p, 2 * h], o, mask=row == b)
                pltpu.store(lhs_sc.at[p, 2 * h + 1], o, mask=row == b + B)
            return carry

        lax.fori_loop(0, NU, unit, 0)

        lhs = [
            jnp.concatenate([lhs_sc[p, j] for j in range(HQ)], axis=1).astype(jnp.bfloat16)
            for p in range(2)
        ]

        def emit(p, band):
            nparts = OS + (LAST_SPLIT - 1 if (p == 1 and band == NBAND - 1) else 0)
            r = res_sc[p, band * OS]
            for s in range(1, nparts):
                r = r + res_sc[p, band * OS + s]
            r4 = r[0:B] + r[B:2 * B]
            for j in range(WG):
                n0 = p * D + j * WR + band * 8
                out_sc[:, n0:n0 + 8] = r4[:, j * 8:(j + 1) * 8]

        order = [(0, g) for g in range(SKEW)]
        for g in range(NO):
            order.append((1, g))
            if g + SKEW < NO:
                order.append((0, g + SKEW))

        pending = []
        for p, g in order:
            s = g % OS
            width = LASTC if (p == 1 and g == NO - 1) else OSC
            for k, c0 in enumerate(range(0, OSC, width)):
                wait_all(wobuf.at[g, p, :, :, pl.ds(c0, width)], wosem.at[wo_sem(g, p, c0)])
                if p == 1 and g + OLA < NO:
                    issue_wo(g + OLA)
                for args in pending:
                    emit(*args)
                pending = []
                w = wobuf[g, p, :, :, c0:c0 + width].reshape(WG * 8, width)
                col = s * OSC + c0
                res_sc[p, g + k] = lax.dot_general(
                    lhs[p][:, col:col + width], w, _NT, preferred_element_type=jnp.float32)
            if s == OS - 1:
                pending.append((p, g // OS))
        for args in pending:
            emit(*args)
        o_ref[...] = out_sc[...].astype(o_ref.dtype)

    hbm = pl.BlockSpec(memory_space=pltpu.HBM)
    bf16, f32 = jnp.bfloat16, jnp.float32
    out = pl.pallas_call(
        kernel,
        in_specs=[hbm] * 10,
        out_specs=pl.BlockSpec(memory_space=pltpu.VMEM),
        out_shape=jax.ShapeDtypeStruct((B, 2 * D), A_x.dtype),
        scratch_shapes=[
            pltpu.VMEM((2, B, D), bf16),
            pltpu.VMEM((2, NHB, WG, WR, HC), bf16),
            pltpu.VMEM((NO, 2, WG, 8, OSC), bf16),
            pltpu.VMEM((NS, 2, HB, CH, DH), bf16),
            pltpu.VMEM((NHB, HB, 8, DH), bf16),
            pltpu.VMEM((2, HQ, 8, DH), f32),
            pltpu.VMEM((B, 2 * D), f32),
            pltpu.VMEM((2, NO + LAST_SPLIT - 1, 8, WG * 8), f32),
            pltpu.SemaphoreType.DMA((2,)),
            pltpu.SemaphoreType.DMA((NQ,)),
            pltpu.SemaphoreType.DMA((2 * NO + LAST_SPLIT - 1,)),
            pltpu.SemaphoreType.DMA((NS,)),
        ],
        compiler_params=pltpu.CompilerParams(
            vmem_limit_bytes=64 * 1024 * 1024,
            disable_bounds_checks=True,
            disable_semaphore_checks=True,
        ),
    )(
        A_x.reshape(B, D), A_k_cache, A_v_cache,
        A_wq.reshape(WG, WR, N), A_wo.T.reshape(WG, WR, N),
        B_x.reshape(B, D), B_k_cache, B_v_cache,
        B_wq.reshape(WG, WR, N), B_wo.T.reshape(WG, WR, N),
    )
    return out.reshape(B, SQ, 2 * D)
```

```python
import jax
import jax.numpy as jnp
from jax import lax
import jax.experimental.pallas as pl
import jax.experimental.pallas.tpu as pltpu

_NT = (((1,), (1,)), ((), ()))

HQ = 32
DH = 128
RPD = 8
CH = 128
LA = 3
NS = LA + 1
WG = 9
QC = 128
QS = 2
OC = 256
OS = 2
OLA = 6
SKEW = 3
FW = 1024
F0POS = 2


@jax.jit
def pallas_concat_heads__sliding_block_cached__sliding_block_cached__decode_kernel(
    A_x: jax.Array,
    A_k_cache: jax.Array,
    A_v_cache: jax.Array,
    A_wq: jax.Array,
    A_wo: jax.Array,
    B_x: jax.Array,
    B_k_cache: jax.Array,
    B_v_cache: jax.Array,
    B_wq: jax.Array,
    B_wo: jax.Array,
):
    B, SQ, D = A_x.shape
    _, HKV, SK, _ = A_k_cache.shape
    N = HQ * DH
    W = min(4096, max(256, SK // 4))
    assert SQ == 1 and HQ == 2 * HKV and 2 * B == 8 and CH == DH
    scale = DH ** -0.5

    UPP = B // 2
    NU = 2 * UPP
    NC = W // CH
    NT = 2 * NC
    WR = D // WG
    NBAND = WR // 8
    HC = N // QS
    HPB = HC // (2 * DH)
    NQ = NBAND * QS
    OSC = N // OS
    NO = NBAND * OS
    OPER = OLA // LA
    HALF = N // 2
    NF = HALF // FW
    assert NT % NS == 0 and OLA % LA == 0 and SKEW < OLA and ((WG - 1) * WR) % 128 == 0

    def kernel(ax, ak, av, awq, awo, bx, bk, bv, bwq, bwo, o_ref,
               xbuf, wqbuf, wobuf, wfbuf, kvbuf, s_sc, q_sc, lhs_sc, out_sc, res_sc,
               xsem, wqsem, wosem, kvsem):
        xs, ks, vs, wqs, wos = (ax, bx), (ak, bk), (av, bv), (awq, bwq), (awo, bwo)

        def wait_all(view, sem):
            pltpu.make_async_copy(view, view, sem).wait()

        def issue_kv(p, u, t):
            src = (ks, vs)[t // NC][p]
            row0 = SK - W + (t % NC) * CH
            for r0 in range(0, CH, RPD):
                for th in range(2):
                    pltpu.make_async_copy(
                        src.at[2 * u + th, :, pl.ds(row0 + r0, RPD), :],
                        kvbuf.at[t % NS, th, :, pl.ds(r0, RPD), :],
                        kvsem.at[t % NS],
                    ).start(priority=th)

        def issue_wq(g):
            rr, s = (g // QS) * 8, g % QS
            for c0 in range(0, HC, QC):
                for p in range(2):
                    pltpu.make_async_copy(
                        wqs[p].at[:, pl.ds(rr, 8), pl.ds(s * HC + c0, QC)],
                        wqbuf.at[p, s, :, pl.ds(rr, 8), pl.ds(c0, QC)],
                        wqsem.at[g],
                    ).start(priority=p)

        def wo_groups(p):
            return WG if p == 1 else WG - 1

        def issue_wo(g):
            if g == NO:
                for c0 in range(0, HALF, FW):
                    for band in range(NBAND):
                        for th in range(2):
                            col = th * HALF + c0
                            pltpu.make_async_copy(
                                awo.at[WG - 1, pl.ds(band * 8, 8), pl.ds(col, FW)],
                                wfbuf.at[pl.ds(band * 8, 8), pl.ds(col, FW)],
                                wosem.at[2 * NO + th * (1 + c0 // FW)],
                            ).start(priority=th)
                return
            band, s = g // OS, g % OS
            for c0 in range(0, OSC, OC):
                for th, p in enumerate((1, 0)):
                    ng = wo_groups(p)
                    pltpu.make_async_copy(
                        wos[p].at[pl.ds(0, ng), pl.ds(band * 8, 8), pl.ds(s * OSC + c0, OC)],
                        wobuf.at[g, p, pl.ds(0, ng), :, pl.ds(c0, OC)],
                        wosem.at[2 * g + p],
                    ).start(priority=th)

        row = lax.broadcasted_iota(jnp.int32, (8, DH), 0)

        def qproj(p, blk):
            x = xbuf[p].astype(jnp.float32)
            x8 = jnp.concatenate([x, x], axis=0).astype(jnp.bfloat16)
            wq = wqbuf[p, blk].reshape(D, HC)
            q = jnp.dot(x8, wq, preferred_element_type=jnp.float32)
            for hh in range(HPB):
                q0 = q[:, (2 * hh) * DH:(2 * hh + 1) * DH]
                q1 = q[:, (2 * hh + 1) * DH:(2 * hh + 2) * DH]
                q_sc[p, blk * HPB + hh] = jnp.where(row < B, q0, q1).astype(jnp.bfloat16)

        for g in range(LA):
            issue_wq(g)
        xcopies = [pltpu.make_async_copy(xs[p], xbuf.at[p], xsem.at[p]) for p in range(2)]
        for p in range(2):
            xcopies[p].start(priority=p)
        lhs_sc[...] = jnp.zeros_like(lhs_sc)
        for g in range(NQ):
            wait_all(wqbuf.at[:, g % QS, :, pl.ds((g // QS) * 8, 8), :], wqsem.at[g])
            if g + LA < NQ:
                issue_wq(g + LA)
            else:
                issue_kv(0, 0, g + LA - NQ)
        for p in range(2):
            xcopies[p].wait()
        for blk in range(QS):
            qproj(0, blk)

        def unit(u, carry):
            p = u // UPP
            b0 = (u % UPP) * 2
            first = (row % B) == b0

            mx, ls, accs = [None] * HKV, [None] * HKV, [None] * HKV
            for t in range(NT):
                c = t % NC
                slot = t % NS
                wait_all(kvbuf.at[slot], kvsem.at[slot])

                tn = t + LA
                if tn < NT:
                    @pl.when(u < UPP)
                    def _():
                        issue_kv(0, u, tn)

                    @pl.when(u >= UPP)
                    def _():
                        issue_kv(1, u - UPP, tn)
                else:
                    tn -= NT

                    @pl.when(u + 1 < UPP)
                    def _():
                        issue_kv(0, u + 1, tn)

                    @pl.when((u + 1 >= UPP) & (u + 1 < NU))
                    def _():
                        issue_kv(1, u + 1 - UPP, tn)

                    @pl.when(u + 1 == NU)
                    def _():
                        for g in range(tn * OPER, (tn + 1) * OPER):
                            issue_wo(g)

                if t < NC:
                    for h in range(HKV):
                        q = q_sc[p, h]
                        s0 = lax.dot_general(q, kvbuf[slot, 0, h], _NT,
                                             preferred_element_type=jnp.float32)
                        s1 = lax.dot_general(q, kvbuf[slot, 1, h], _NT,
                                             preferred_element_type=jnp.float32)
                        sc = jnp.where(first, s0, s1)
                        s_sc[h, c] = sc
                        mx[h] = sc if c == 0 else jnp.maximum(mx[h], sc)
                        if c == NC - 1:
                            mx[h] = jnp.max(mx[h], axis=-1, keepdims=True)
                else:
                    if c % 2 == 1 and c // 2 < QS:
                        @pl.when(u == 0)
                        def _():
                            qproj(1, c // 2)

                    for h in range(HKV):
                        e = jnp.exp((s_sc[h, c] - mx[h]) * scale)
                        ls[h] = e if c == 0 else ls[h] + e
                        pb = e.astype(jnp.bfloat16)
                        pv0 = jnp.dot(pb, kvbuf[slot, 0, h], preferred_element_type=jnp.float32)
                        pv1 = jnp.dot(pb, kvbuf[slot, 1, h], preferred_element_type=jnp.float32)
                        pv = jnp.where(first, pv0, pv1)
                        accs[h] = pv if c == 0 else accs[h] + pv

            for h in range(HKV):
                o = accs[h] / jnp.sum(ls[h], axis=-1, keepdims=True)
                pltpu.store(lhs_sc.at[p, 2 * h], o, mask=(row == b0) | (row == b0 + 1))
                pltpu.store(lhs_sc.at[p, 2 * h + 1], o,
                            mask=(row == b0 + B) | (row == b0 + B + 1))
            return carry

        lax.fori_loop(0, NU, unit, 0)

        lhs = [
            jnp.concatenate([lhs_sc[p, j] for j in range(HQ)], axis=1).astype(jnp.bfloat16)
            for p in range(2)
        ]

        def emit(p, band):
            ng = wo_groups(p)
            r = res_sc[p, band * OS, :, 0:ng * 8]
            for s in range(1, OS):
                r = r + res_sc[p, band * OS + s, :, 0:ng * 8]
            r4 = r[0:B] + r[B:2 * B]
            for j in range(ng):
                n0 = p * D + j * WR + band * 8
                out_sc[:, n0:n0 + 8] = r4[:, j * 8:(j + 1) * 8]

        order = [(1, g) for g in range(SKEW)]
        for g in range(NO):
            if g == NO - F0POS:
                order.append((2, 0))
            order.append((0, g))
            if g + SKEW < NO:
                order.append((1, g + SKEW))
        order += [(2, 1 + k) for k in range(NF)]

        pending = []
        for p, g in order:
            if p == 2:
                c0, width = (0, HALF) if g == 0 else (HALF + (g - 1) * FW, FW)
                wait_all(wfbuf.at[:, pl.ds(c0, width)], wosem.at[2 * NO + g])
            else:
                ng = wo_groups(p)
                wait_all(wobuf.at[g, p, pl.ds(0, ng)], wosem.at[2 * g + p])
                if p == 0 and g + OLA <= NO:
                    issue_wo(g + OLA)
            for args in pending:
                emit(*args)
            pending = []
            if p == 2:
                res_sc[0, NO + g, :, 0:WR] = lax.dot_general(
                    lhs[0][:, c0:c0 + width], wfbuf[:, c0:c0 + width], _NT,
                    preferred_element_type=jnp.float32)
            else:
                s = g % OS
                w = wobuf[g, p, 0:ng].reshape(ng * 8, OSC)
                res_sc[p, g, :, 0:ng * 8] = lax.dot_general(
                    lhs[p][:, s * OSC:(s + 1) * OSC], w, _NT,
                    preferred_element_type=jnp.float32)
                if s == OS - 1:
                    pending.append((p, g // OS))
        assert not pending
        r = res_sc[0, NO, :, 0:WR]
        for k in range(NF):
            r = r + res_sc[0, NO + 1 + k, :, 0:WR]
        out_sc[:, (WG - 1) * WR:WG * WR] = r[0:B] + r[B:2 * B]
        o_ref[...] = out_sc[...].astype(o_ref.dtype)

    hbm = pl.BlockSpec(memory_space=pltpu.HBM)
    bf16, f32 = jnp.bfloat16, jnp.float32
    out = pl.pallas_call(
        kernel,
        in_specs=[hbm] * 10,
        out_specs=pl.BlockSpec(memory_space=pltpu.VMEM),
        out_shape=jax.ShapeDtypeStruct((B, 2 * D), A_x.dtype),
        scratch_shapes=[
            pltpu.VMEM((2, B, D), bf16),
            pltpu.VMEM((2, QS, WG, WR, HC), bf16),
            pltpu.VMEM((NO, 2, WG, 8, OSC), bf16),
            pltpu.VMEM((WR, N), bf16),
            pltpu.VMEM((NS, 2, HKV, CH, DH), bf16),
            pltpu.VMEM((HKV, NC, 8, CH), f32),
            pltpu.VMEM((2, HKV, 8, DH), bf16),
            pltpu.VMEM((2, HQ, 8, DH), f32),
            pltpu.VMEM((B, 2 * D), f32),
            pltpu.VMEM((2, NO + 1 + NF, 8, WG * 8), f32),
            pltpu.SemaphoreType.DMA((2,)),
            pltpu.SemaphoreType.DMA((NQ,)),
            pltpu.SemaphoreType.DMA((2 * NO + 1 + NF,)),
            pltpu.SemaphoreType.DMA((NS,)),
        ],
        compiler_params=pltpu.CompilerParams(
            vmem_limit_bytes=64 * 1024 * 1024,
            disable_bounds_checks=True,
            disable_semaphore_checks=True,
        ),
    )(
        A_x.reshape(B, D), A_k_cache, A_v_cache,
        A_wq.reshape(WG, WR, N), A_wo.T.reshape(WG, WR, N),
        B_x.reshape(B, D), B_k_cache, B_v_cache,
        B_wq.reshape(WG, WR, N), B_wo.T.reshape(WG, WR, N),
    )
    return out.reshape(B, SQ, 2 * D)
```
